```python
import jax
import jax.numpy as jnp

def _softmax(x, axis=-1):
    return jax.nn.softmax(x, axis=axis)
def _gelu(x):
    return jax.nn.gelu(x, approximate=True)
def _silu(x):
    return jax.nn.silu(x)
def _sigmoid(x):
    return jax.nn.sigmoid(x)
def _layernorm(x, axis=-1, eps=1e-5):
    m = jnp.mean(x, axis=axis, keepdims=True)
    v = jnp.var(x, axis=axis, keepdims=True)
    return (x - m) / jnp.sqrt(v + eps)
def _scatter_add(tgt, idx, src, axis=0):
    return tgt.at[idx].add(src)
def _segment_sum(src, seg, n):
    return jax.ops.segment_sum(src, seg, n)
class _Rng:
    def __init__(self, key):
        self._k = key
    def _next(self):
        self._k, sub = jax.random.split(self._k)
        return sub
    def normal(self, shape):
        return jax.random.normal(self._next(), shape, dtype=jnp.bfloat16)
    def randint(self, lo, hi, shape):
        return jax.random.randint(self._next(), shape, lo, hi, dtype=jnp.int32)
    def uniform(self, shape, lo=0.0, hi=1.0):
        return jax.random.uniform(self._next(), shape, jnp.bfloat16, lo, hi)
    def permutation(self, n):
        return jax.random.permutation(self._next(), n)


kernel_name = 'parallel_sum__gqa_block_cached__moe_arch_mod__decode'

def setup_inputs():
    _rng = _Rng(jax.random.key(int.from_bytes(__import__("os").urandom(4), "little")))
    _w = (lambda a: (lambda t: t.astype(jnp.bfloat16) if jnp.issubdtype(t.dtype, jnp.floating) else t)(jnp.asarray(a)))
    def _A_setup():
        B, Sq, D = 1, 1, 448
        Hq, Hkv, Sk, Dh = 16, 8, 65536, 256
        assert Hq % Hkv == 0, (Hq, Hkv)
        return {
            "x": _w((lambda *s: _rng.normal(s) * 0.05)(B, Sq, D)),
            "k_cache": _w((lambda *s: _rng.normal(s) * 0.05)(B, Hkv, Sk, Dh)),
            "v_cache": _w((lambda *s: _rng.normal(s) * 0.05)(B, Hkv, Sk, Dh)),
            "wq": _w((lambda *s: _rng.normal(s) * 0.05)(D, Hq * Dh) * (D ** -0.5)),
            "wo": _w((lambda *s: _rng.normal(s) * 0.05)(Hq * Dh, D) * ((Hq * Dh) ** -0.5)),
        }
    _A_in = _A_setup()

    def _B_setup():
        B, S, D, F, C = 1, 1, 448, 1792, 1
        return {
            "x": _w((lambda *s: _rng.normal(s) * 0.05)(B, S, D)),
            "w_r": _w((lambda *s: _rng.normal(s) * 0.05)(D)),
            "w_gate": _w((lambda *s: _rng.normal(s) * 0.05)(D, F)),
            "w_up": _w((lambda *s: _rng.normal(s) * 0.05)(D, F)),
            "w_down": _w((lambda *s: _rng.normal(s) * 0.05)(F, D)),
        }
    _B_in = _B_setup()

    return {
        "A_x": _A_in["x"],
        "A_k_cache": _A_in["k_cache"],
        "A_v_cache": _A_in["v_cache"],
        "A_wq": _A_in["wq"],
        "A_wo": _A_in["wo"],
        "B_x": _B_in["x"],
        "B_w_r": _B_in["w_r"],
        "B_w_gate": _B_in["w_gate"],
        "B_w_up": _B_in["w_up"],
        "B_w_down": _B_in["w_down"],
    }

def reference(A_x, A_k_cache, A_v_cache, A_wq, A_wo, B_x, B_w_r, B_w_gate, B_w_up, B_w_down):
    def _A_ref(x, k_cache, v_cache, wq, wo):
        B, Sq, D = x.shape
        Hq, Dh = 16, 256
        Hkv = k_cache.shape[1]
        rep = Hq // Hkv
        q = (lambda x, *d: x.transpose(*d))((x @ wq).reshape(B, Sq, Hq, Dh), 0, 2, 1, 3)
        k = jnp.repeat(k_cache, rep, axis=1)
        v = jnp.repeat(v_cache, rep, axis=1)
        scores = jnp.einsum("bhqd,bhkd->bhqk", q, k) * (Dh ** -0.5)
        p = _softmax(scores, axis=-1)
        o = jnp.einsum("bhqk,bhkd->bhqd", p, v)
        return (lambda x, *d: x.transpose(*d))(o, 0, 2, 1, 3).reshape(B, Sq, Hq * Dh) @ wo

    def _B_ref(x, w_r, w_gate, w_up, w_down):
        B, S, D = x.shape
        C = 1
        r = x @ w_r
        idx = jnp.argsort(-r, axis=-1)[:, :C]
        idx_e = jnp.repeat(idx.reshape(B, C, 1), D, axis=2)
        x_sel = jnp.take_along_axis(x, idx_e, axis=1)
        g = _silu(x_sel @ w_gate)
        u = x_sel @ w_up
        y = (g * u) @ w_down
        r_sel = _sigmoid(jnp.take_along_axis(r, idx, axis=1))
        y = y * r_sel.reshape(B, C, 1)
        b_off = (jnp.arange(B) * S).reshape(B, 1)
        flat_idx = (idx + b_off).reshape(B * C)
        zero = (x * 0.0).reshape(B * S, D)
        upd = _scatter_add(zero, flat_idx, y.reshape(B * C, D), axis=0)
        return x + upd.reshape(B, S, D)

    x = A_x
    xn = _layernorm(x, axis=-1)
    return x + _A_ref(xn, A_k_cache, A_v_cache, A_wq, A_wo) + _B_ref(xn, B_w_r, B_w_gate, B_w_up, B_w_down)
```

```python
import functools

import jax
import jax.numpy as jnp
import jax.experimental.pallas as pl
import jax.experimental.pallas.tpu as pltpu

_HQ = 16
_DH = 256
_EPS = 1e-5

_BLK = 2048
_NBUF = 5
_DMA_ROWS = 96
_WROWS = 32


def _split(total, step):
    out, o = [], 0
    while o < total:
        n = min(step, total - o)
        out.append((o, n))
        o += n
    return out


def _bf(x):
    return x.astype(jnp.bfloat16).astype(jnp.float32)


def _dot_t(a, b):
    return jax.lax.dot_general(a, b, (((1,), (1,)), ((), ())), preferred_element_type=jnp.float32)


def _kernel(x_ref, wr_ref, k_hbm, v_hbm, wq_hbm, wo_hbm, wg_hbm, wu_hbm, wd_hbm, o_ref,
            kbuf, vbuf, wq_ref, wo_ref, wg_ref, wu_ref, wd_ref, q_ref, acc_ref,
            kv_sem, w_sem, *, blk, nbuf, dma_rows):
    _, hkv, sk, dh = k_hbm.shape
    d = x_ref.shape[-1]
    rep = _HQ // hkv
    nblk_h = sk // blk
    nblk = hkv * nblk_h
    subs = _split(blk, dma_rows)
    f32, bf16 = jnp.float32, jnp.bfloat16

    def start_kv(i, slot):
        h = i // nblk_h
        base = pl.multiple_of((i % nblk_h) * blk, blk)
        for o, n in subs:
            pltpu.make_async_copy(k_hbm.at[0, h, pl.ds(base + o, n)],
                                  kbuf.at[slot, pl.ds(o, n)], kv_sem.at[0, slot]).start(priority=0)
            pltpu.make_async_copy(v_hbm.at[0, h, pl.ds(base + o, n)],
                                  vbuf.at[slot, pl.ds(o, n)], kv_sem.at[1, slot]).start(priority=1)

    def start_w(src, dst, sem_idx, rows):
        for c, (o, n) in enumerate(_split(src.shape[0], rows)):
            pltpu.make_async_copy(src.at[pl.ds(o, n)], dst.at[pl.ds(o, n)],
                                  w_sem.at[sem_idx]).start(priority=c % 2)

    def wait_w(dst, sem_idx):
        pltpu.make_async_copy(dst, dst, w_sem.at[sem_idx]).wait()

    start_w(wq_hbm, wq_ref, 0, 16)
    for j in range(nbuf):
        start_kv(j, j)
    start_w(wg_hbm, wg_ref, 1, 16)
    start_w(wu_hbm, wu_ref, 2, 16)
    start_w(wd_hbm, wd_ref, 3, 16)
    start_w(wo_hbm, wo_ref, 4, 16)

    x = x_ref[0].astype(f32)
    mean = jnp.mean(x, axis=-1, keepdims=True)
    var = jnp.mean(jnp.square(x - mean), axis=-1, keepdims=True)
    xn = _bf(_bf(x - _bf(mean)) / _bf(jnp.sqrt(_bf(_bf(var) + _EPS))))
    xn8 = jnp.broadcast_to(xn, (8, d)).astype(bf16)

    wait_w(wq_ref, 0)
    row = jax.lax.broadcasted_iota(jnp.int32, (8, dh), 0)
    for h in range(hkv):
        qh = jnp.dot(xn8, wq_ref[:, h * rep * dh:(h + 1) * rep * dh],
                     preferred_element_type=f32)
        sel = qh[:, 0:dh]
        for r in range(1, rep):
            sel = jnp.where(row % rep == r, qh[:, r * dh:(r + 1) * dh], sel)
        q_ref[h] = sel.astype(bf16)

    def ffn():
        wait_w(wg_ref, 1)
        wait_w(wu_ref, 2)
        wait_w(wd_ref, 3)
        g = _bf(jnp.dot(xn8, wg_ref[...], preferred_element_type=f32))
        u = _bf(jnp.dot(xn8, wu_ref[...], preferred_element_type=f32))
        g = _bf(g * jax.nn.sigmoid(g))
        y = _bf(_dot_t((g * u).astype(bf16), wd_ref[...]))
        r = _bf(jnp.sum(xn * wr_ref[...].astype(f32).reshape(1, d), axis=-1, keepdims=True))
        y = _bf(y * _bf(jax.nn.sigmoid(r)))
        acc_ref[...] = jnp.zeros(acc_ref.shape, f32)
        return xn * 0.0 + y

    def body(i, carry):
        m, l, acc = carry
        slot = i % nbuf
        h = i // nblk_h
        j = i % nblk_h
        first = j == 0
        m = jnp.where(first, -jnp.inf, m)
        l = jnp.where(first, 0.0, l)
        acc = jnp.where(first, 0.0, acc)

        pltpu.make_async_copy(kbuf.at[slot], kbuf.at[slot], kv_sem.at[0, slot]).wait()
        s = _dot_t(q_ref[h], kbuf[slot]) * (dh ** -0.5)
        m_new = jnp.maximum(m, jnp.max(s, axis=-1, keepdims=True))
        alpha = jnp.exp(m - m_new)
        p = jnp.exp(s - m_new)
        l = alpha * l + jnp.sum(p, axis=-1, keepdims=True)
        pltpu.make_async_copy(vbuf.at[slot], vbuf.at[slot], kv_sem.at[1, slot]).wait()
        acc = alpha * acc + jnp.dot(p.astype(bf16), vbuf[slot], preferred_element_type=f32)

        @pl.when(i + nbuf < nblk)
        def _():
            start_kv(i + nbuf, slot)

        @pl.when(j == nblk_h - 1)
        def _():
            @pl.when(h == 0)
            def _():
                wait_w(wo_ref, 4)
            o = acc / l
            lhs = jnp.concatenate(
                [jnp.broadcast_to(o[r:r + 1], (8, dh)) for r in range(rep)], axis=1).astype(bf16)
            w = wo_ref[:, pl.ds(pl.multiple_of(h * rep * dh, rep * dh), rep * dh)]
            acc_ref[...] += _dot_t(lhs, w)

        return m_new, l, acc

    upd = ffn()
    init = (jnp.zeros((8, 1), f32), jnp.zeros((8, 1), f32), jnp.zeros((8, dh), f32))
    jax.lax.fori_loop(0, nblk, body, init)

    a = _bf(acc_ref[0:1, :])
    o_ref[0] = (_bf(x + a) + _bf(xn + upd[0:1])).astype(o_ref.dtype)


@jax.jit
def pallas_parallel_sum__gqa_block_cached__moe_arch_mod__decode_kernel(
    A_x: jax.Array,
    A_k_cache: jax.Array,
    A_v_cache: jax.Array,
    A_wq: jax.Array,
    A_wo: jax.Array,
    B_x: jax.Array,
    B_w_r: jax.Array,
    B_w_gate: jax.Array,
    B_w_up: jax.Array,
    B_w_down: jax.Array,
):
    del B_x
    b, sq, d = A_x.shape
    _, hkv, sk, dh = A_k_cache.shape
    f = B_w_gate.shape[1]
    assert b == 1 and sq == 1 and dh == _DH and sk % _BLK == 0 and _HQ % hkv == 0
    bf16 = jnp.bfloat16
    any_spec = pl.BlockSpec(memory_space=pltpu.HBM)
    vmem_spec = pl.BlockSpec(memory_space=pltpu.VMEM)
    return pl.pallas_call(
        functools.partial(_kernel, blk=_BLK, nbuf=_NBUF, dma_rows=_DMA_ROWS),
        in_specs=[vmem_spec, vmem_spec] + [any_spec] * 7,
        out_specs=vmem_spec,
        out_shape=jax.ShapeDtypeStruct(A_x.shape, A_x.dtype),
        scratch_shapes=[
            pltpu.VMEM((_NBUF, _BLK, dh), bf16),
            pltpu.VMEM((_NBUF, _BLK, dh), bf16),
            pltpu.VMEM(A_wq.shape, bf16),
            pltpu.VMEM(A_wo.shape[::-1], bf16),
            pltpu.VMEM(B_w_gate.shape, bf16),
            pltpu.VMEM(B_w_up.shape, bf16),
            pltpu.VMEM(B_w_down.shape[::-1], bf16),
            pltpu.VMEM((hkv, 8, dh), bf16),
            pltpu.VMEM((8, d), jnp.float32),
            pltpu.SemaphoreType.DMA((2, _NBUF)),
            pltpu.SemaphoreType.DMA((5,)),
        ],
        compiler_params=pltpu.CompilerParams(vmem_limit_bytes=64 * 2**20),
    )(A_x, B_w_r, A_k_cache, A_v_cache, A_wq, A_wo.T, B_w_gate, B_w_up, B_w_down.T)
```

```python
import functools

import jax
import jax.numpy as jnp
import jax.experimental.pallas as pl
import jax.experimental.pallas.tpu as pltpu

_HQ = 16
_DH = 256
_EPS = 1e-5

_BLK = 4096
_NBUF = 3
_DMA_ROWS = 96
_WCOLS = 1024


def _split(total, step):
    out, o = [], 0
    while o < total:
        n = min(step, total - o)
        out.append((o, n))
        o += n
    return out


def _bf(x):
    return x.astype(jnp.bfloat16).astype(jnp.float32)


def _dot_t(a, b):
    return jax.lax.dot_general(a, b, (((1,), (1,)), ((), ())), preferred_element_type=jnp.float32)


def _kernel(x_hbm, wr_hbm, k_hbm, v_hbm, wq_hbm, wo_hbm, wg_hbm, wu_hbm, wd_hbm, o_ref,
            x_ref, wr_ref, kbuf, vbuf, wq_ref, wo_ref, wg_ref, wu_ref, wd_ref, q_ref, acc_ref,
            kv_sem, w_sem, *, blk, nbuf, dma_rows):
    _, hkv, sk, dh = k_hbm.shape
    d = x_hbm.shape[-1]
    rep = _HQ // hkv
    nblk_h = sk // blk
    nblk = hkv * nblk_h
    subs = _split(blk, dma_rows)
    f32, bf16 = jnp.float32, jnp.bfloat16

    def start_kv(i, slot):
        h = i // nblk_h
        base = pl.multiple_of((i % nblk_h) * blk, blk)
        for o, n in subs:
            pltpu.make_async_copy(k_hbm.at[0, h, pl.ds(base + o, n)],
                                  kbuf.at[slot, pl.ds(o, n)], kv_sem.at[0, slot]).start(priority=0)
            pltpu.make_async_copy(v_hbm.at[0, h, pl.ds(base + o, n)],
                                  vbuf.at[slot, pl.ds(o, n)], kv_sem.at[1, slot]).start(priority=1)

    def start_w(src, dst, sem_idx):
        c = 0
        for o, n in _split(src.shape[0], 16):
            for co, cn in _split(src.shape[1], _WCOLS):
                pltpu.make_async_copy(src.at[pl.ds(o, n), pl.ds(co, cn)],
                                      dst.at[pl.ds(o, n), pl.ds(co, cn)],
                                      w_sem.at[sem_idx]).start(priority=c % 2)
                c += 1

    def wait_w(dst, sem_idx):
        pltpu.make_async_copy(dst, dst, w_sem.at[sem_idx]).wait()

    x_cp = pltpu.make_async_copy(x_hbm, x_ref, w_sem.at[5])
    wr_cp = pltpu.make_async_copy(wr_hbm, wr_ref, w_sem.at[6])
    x_cp.start(priority=0)
    wr_cp.start(priority=1)
    start_w(wq_hbm, wq_ref, 0)
    for j in range(nbuf):
        start_kv(j, j)
    start_w(wg_hbm, wg_ref, 1)
    start_w(wu_hbm, wu_ref, 2)
    start_w(wo_hbm, wo_ref, 4)

    x_cp.wait()
    x = x_ref[0].astype(f32)
    mean = jnp.mean(x, axis=-1, keepdims=True)
    var = jnp.mean(jnp.square(x - mean), axis=-1, keepdims=True)
    xn = _bf(_bf(x - _bf(mean)) / _bf(jnp.sqrt(_bf(_bf(var) + _EPS))))
    xn8 = jnp.broadcast_to(xn, (8, d)).astype(bf16)

    wait_w(wq_ref, 0)
    row = jax.lax.broadcasted_iota(jnp.int32, (8, dh), 0)
    for h in range(hkv):
        qh = jnp.dot(xn8, wq_ref[:, h * rep * dh:(h + 1) * rep * dh],
                     preferred_element_type=f32)
        sel = qh[:, 0:dh]
        for r in range(1, rep):
            sel = jnp.where(row % rep == r, qh[:, r * dh:(r + 1) * dh], sel)
        q_ref[h] = sel.astype(bf16)

    def ffn():
        wait_w(wg_ref, 1)
        wait_w(wu_ref, 2)
        wr_cp.wait()
        g = _bf(jnp.dot(xn8, wg_ref[...], preferred_element_type=f32))
        u = _bf(jnp.dot(xn8, wu_ref[...], preferred_element_type=f32))
        g = _bf(g * jax.nn.sigmoid(g))
        r = _bf(jnp.sum(xn * wr_ref[...].astype(f32).reshape(1, d), axis=-1, keepdims=True))
        return (g * u).astype(bf16), _bf(jax.nn.sigmoid(r))

    def body(i, carry):
        m, l, acc = carry
        slot = i % nbuf
        h = i // nblk_h
        j = i % nblk_h
        first = j == 0
        m = jnp.where(first, -jnp.inf, m)
        l = jnp.where(first, 0.0, l)
        acc = jnp.where(first, 0.0, acc)

        pltpu.make_async_copy(kbuf.at[slot], kbuf.at[slot], kv_sem.at[0, slot]).wait()
        s = _dot_t(q_ref[h], kbuf[slot]) * (dh ** -0.5)
        m_new = jnp.maximum(m, jnp.max(s, axis=-1, keepdims=True))
        alpha = jnp.exp(m - m_new)
        p = jnp.exp(s - m_new)
        l = alpha * l + jnp.sum(p, axis=-1, keepdims=True)
        pltpu.make_async_copy(vbuf.at[slot], vbuf.at[slot], kv_sem.at[1, slot]).wait()
        acc = alpha * acc + jnp.dot(p.astype(bf16), vbuf[slot], preferred_element_type=f32)

        @pl.when(i + nbuf < nblk)
        def _():
            start_kv(i + nbuf, slot)

        @pl.when(i + nbuf == nblk)
        def _():
            start_w(wd_hbm, wd_ref, 3)

        @pl.when(j == nblk_h - 1)
        def _():
            @pl.when(h == 0)
            def _():
                wait_w(wo_ref, 4)
            o = acc / l
            lhs = jnp.concatenate(
                [jnp.broadcast_to(o[r:r + 1], (8, dh)) for r in range(rep)], axis=1).astype(bf16)
            w = wo_ref[:, pl.ds(pl.multiple_of(h * rep * dh, rep * dh), rep * dh)]
            acc_ref[...] += _dot_t(lhs, w)

        return m_new, l, acc

    hid, gate = ffn()
    acc_ref[...] = jnp.zeros(acc_ref.shape, f32)
    init = (jnp.zeros((8, 1), f32), jnp.zeros((8, 1), f32), jnp.zeros((8, dh), f32))
    jax.lax.fori_loop(0, nblk, body, init)

    a = _bf(acc_ref[0:1, :])
    wait_w(wd_ref, 3)
    y = _bf(_bf(_dot_t(hid, wd_ref[...])) * gate)
    upd = xn * 0.0 + y
    o_ref[0] = (_bf(x + a) + _bf(xn + upd[0:1])).astype(o_ref.dtype)


@jax.jit
def pallas_parallel_sum__gqa_block_cached__moe_arch_mod__decode_kernel(
    A_x: jax.Array,
    A_k_cache: jax.Array,
    A_v_cache: jax.Array,
    A_wq: jax.Array,
    A_wo: jax.Array,
    B_x: jax.Array,
    B_w_r: jax.Array,
    B_w_gate: jax.Array,
    B_w_up: jax.Array,
    B_w_down: jax.Array,
):
    del B_x
    b, sq, d = A_x.shape
    _, hkv, sk, dh = A_k_cache.shape
    f = B_w_gate.shape[1]
    assert b == 1 and sq == 1 and dh == _DH and sk % _BLK == 0 and _HQ % hkv == 0
    bf16 = jnp.bfloat16
    any_spec = pl.BlockSpec(memory_space=pltpu.HBM)
    vmem_spec = pl.BlockSpec(memory_space=pltpu.VMEM)
    return pl.pallas_call(
        functools.partial(_kernel, blk=_BLK, nbuf=_NBUF, dma_rows=_DMA_ROWS),
        in_specs=[any_spec] * 9,
        out_specs=vmem_spec,
        out_shape=jax.ShapeDtypeStruct(A_x.shape, A_x.dtype),
        scratch_shapes=[
            pltpu.VMEM(A_x.shape, bf16),
            pltpu.VMEM(B_w_r.shape, bf16),
            pltpu.VMEM((_NBUF, _BLK, dh), bf16),
            pltpu.VMEM((_NBUF, _BLK, dh), bf16),
            pltpu.VMEM(A_wq.shape, bf16),
            pltpu.VMEM(A_wo.shape[::-1], bf16),
            pltpu.VMEM(B_w_gate.shape, bf16),
            pltpu.VMEM(B_w_up.shape, bf16),
            pltpu.VMEM(B_w_down.shape[::-1], bf16),
            pltpu.VMEM((hkv, 8, dh), bf16),
            pltpu.VMEM((8, d), jnp.float32),
            pltpu.SemaphoreType.DMA((2, _NBUF)),
            pltpu.SemaphoreType.DMA((7,)),
        ],
        compiler_params=pltpu.CompilerParams(vmem_limit_bytes=64 * 2**20),
    )(A_x, B_w_r, A_k_cache, A_v_cache, A_wq, A_wo.T, B_w_gate, B_w_up, B_w_down.T)
```
